```python
import jax
import jax.numpy as jnp

def _softmax(x, axis=-1):
    return jax.nn.softmax(x, axis=axis)

def _gelu(x):
    return jax.nn.gelu(x, approximate=True)

def _silu(x):
    return jax.nn.silu(x)

def _sigmoid(x):
    return jax.nn.sigmoid(x)

def _layernorm(x, axis=-1, eps=1e-05):
    m = jnp.mean(x, axis=axis, keepdims=True)
    v = jnp.var(x, axis=axis, keepdims=True)
    return (x - m) / jnp.sqrt(v + eps)

def _scatter_add(tgt, idx, src, axis=0):
    return tgt.at[idx].add(src)

def _segment_sum(src, seg, n):
    return jax.ops.segment_sum(src, seg, n)

class _Rng:

    def __init__(self, key):
        self._k = key

    def _next(self):
        self._k, sub = jax.random.split(self._k)
        return sub

    def normal(self, shape):
        return jax.random.normal(self._next(), shape, dtype=jnp.bfloat16)

    def randint(self, lo, hi, shape):
        return jax.random.randint(self._next(), shape, lo, hi, dtype=jnp.int32)

    def uniform(self, shape, lo=0.0, hi=1.0):
        return jax.random.uniform(self._next(), shape, jnp.bfloat16, lo, hi)

    def permutation(self, n):
        return jax.random.permutation(self._next(), n)
kernel_name = 'sequential_preLN__ssm_conv_s4__mixer_gmlp__prompt'

def _fwd_setup_inputs():
    _rng = _Rng(jax.random.key(int.from_bytes(__import__("os").urandom(4), "little")))
    _w = lambda a: (lambda t: t.astype(jnp.bfloat16) if jnp.issubdtype(t.dtype, jnp.floating) else t)(jnp.asarray(a))

    def _A_setup():
        B, L, D, N = (1, 2048, 576, 128)
        A_re = -jnp.exp((lambda *s: _rng.normal(s) * 0.05)(D, N))
        A_im = jnp.pi * (lambda *s: _rng.normal(s) * 0.05)(D, N)
        B_re = (lambda *s: _rng.normal(s) * 0.05)(D, N)
        B_im = (lambda *s: _rng.normal(s) * 0.05)(D, N)
        C_re = (lambda *s: _rng.normal(s) * 0.05)(D, N)
        C_im = (lambda *s: _rng.normal(s) * 0.05)(D, N)
        log_dt = (lambda *s: _rng.normal(s) * 0.05)(D) * 0.5 - 4.0
        Dskip = (lambda *s: _rng.normal(s) * 0.05)(D)
        return {'u': _w((lambda *s: _rng.normal(s) * 0.05)(B, L, D)), 'A_re': _w(A_re), 'A_im': _w(A_im), 'B_re': _w(B_re), 'B_im': _w(B_im), 'C_re': _w(C_re), 'C_im': _w(C_im), 'log_dt': _w(log_dt), 'Dskip': _w(Dskip)}
    _A_in = _A_setup()

    def _B_setup():
        B, S, D, F = (1, 2048, 576, 4608)
        Fh = F // 2
        return {'x': _w((lambda *s: _rng.normal(s) * 0.05)(B, S, D)), 'w_in': _w((lambda *s: _rng.normal(s) * 0.05)(D, 2 * Fh)), 'w_sp': _w(0.01 * (lambda *s: _rng.normal(s) * 0.05)(S, S)), 'b_sp': _w(1.0 + 0.01 * (lambda *s: _rng.normal(s) * 0.05)(S)), 'w_out': _w((lambda *s: _rng.normal(s) * 0.05)(Fh, D))}
    _B_in = _B_setup()
    return {'A_u': _A_in['u'], 'A_A_re': _A_in['A_re'], 'A_A_im': _A_in['A_im'], 'A_B_re': _A_in['B_re'], 'A_B_im': _A_in['B_im'], 'A_C_re': _A_in['C_re'], 'A_C_im': _A_in['C_im'], 'A_log_dt': _A_in['log_dt'], 'A_Dskip': _A_in['Dskip'], 'B_x': _B_in['x'], 'B_w_in': _B_in['w_in'], 'B_w_sp': _B_in['w_sp'], 'B_b_sp': _B_in['b_sp'], 'B_w_out': _B_in['w_out']}

def _fwd_reference(A_u, A_A_re, A_A_im, A_B_re, A_B_im, A_C_re, A_C_im, A_log_dt, A_Dskip, B_x, B_w_in, B_w_sp, B_b_sp, B_w_out):

    def _A_ref(u, A_re, A_im, B_re, B_im, C_re, C_im, log_dt, Dskip):
        Bsz, L, D = u.shape
        dt = jnp.exp(log_dt)[:, None]
        A = A_re + 1j * A_im
        Bc = B_re + 1j * B_im
        Cc = C_re + 1j * C_im
        logdA = dt * A
        dB = dt * Bc
        l = (lambda x, dt: x.astype(dt))(jnp.arange(L), A_re.dtype)
        P = jnp.exp(logdA[:, :, None] * l[None, None, :])
        K = jnp.einsum('dn,dnl,dn->dl', Cc, P, dB).real
        L2 = 2 * L
        Kp = jnp.pad(K, ((0, 0), (0, L)))
        up = (lambda x, *d: x.transpose(*d))(u, 0, 2, 1)
        up = jnp.pad(up, ((0, 0), (0, 0), (0, L)))
        Kf = (lambda x, axes=(-2, -1): jnp.fft.rfft2(x.astype(jnp.float32), axes=axes))(Kp[:, None, :], axes=(-2, -1))
        Uf = (lambda x, axes=(-2, -1): jnp.fft.rfft2(x.astype(jnp.float32), axes=axes))(up[:, :, None, :], axes=(-2, -1))
        Yf = Uf * Kf[None, :, :, :]
        y = (lambda x, s, axes=(-2, -1): jnp.fft.irfft2(x, s=s, axes=axes).astype(jnp.bfloat16))(Yf, (1, L2), axes=(-2, -1))[:, :, 0, :L]
        y = (lambda x, *d: x.transpose(*d))(y, 0, 2, 1) + u * Dskip[None, None, :]
        return y

    def _B_ref(x, w_in, w_sp, b_sp, w_out):
        B, S, D = x.shape
        F = w_in.shape[-1]
        Fh = F // 2
        z = _gelu(jnp.einsum('bsd,df->bsf', x, w_in))
        z1 = z[..., :Fh].copy()
        z2 = _layernorm(z[..., Fh:], axis=-1)
        g = jnp.einsum('ts,bsf->btf', w_sp, z2) + b_sp[None, :, None]
        return jnp.einsum('bsf,fd->bsd', z1 * g, w_out)
    x = A_u
    h = x + _A_ref(_layernorm(x, axis=-1), A_A_re, A_A_im, A_B_re, A_B_im, A_C_re, A_C_im, A_log_dt, A_Dskip)
    h2 = h + _B_ref(_layernorm(h, axis=-1), B_w_in, B_w_sp, B_b_sp, B_w_out)
    return h2

def setup_inputs():
    _inp = _fwd_setup_inputs()
    _gk = jax.random.fold_in(jax.random.key(int.from_bytes(__import__("os").urandom(4), "little")), 2 ** 31 - 1)
    _shapes = [[1, 2048, 576]]
    _dtypes = ['bfloat16']
    _gks = jax.random.split(_gk, len(_shapes))
    _gs = [jax.random.normal(k, s, dtype=jnp.dtype(d)) * 0.05 for k, s, d in zip(_gks, _shapes, _dtypes)]
    _inp['grad_out'] = _gs[0]
    return _inp

def reference(A_u, A_A_re, A_A_im, A_B_re, A_B_im, A_C_re, A_C_im, A_log_dt, A_Dskip, B_w_in, B_w_sp, B_b_sp, B_w_out, B_x, grad_out):
    _const = dict(B_x=B_x)

    def _f(*_d):
        return _fwd_reference(**{'A_u': _d[0], 'A_A_re': _d[1], 'A_A_im': _d[2], 'A_B_re': _d[3], 'A_B_im': _d[4], 'A_C_re': _d[5], 'A_C_im': _d[6], 'A_log_dt': _d[7], 'A_Dskip': _d[8], 'B_w_in': _d[9], 'B_w_sp': _d[10], 'B_b_sp': _d[11], 'B_w_out': _d[12], **_const})
    _out, _vjp = jax.vjp(_f, A_u, A_A_re, A_A_im, A_B_re, A_B_im, A_C_re, A_C_im, A_log_dt, A_Dskip, B_w_in, B_w_sp, B_b_sp, B_w_out)
    _grads = _vjp(grad_out)
    _out0 = jnp.asarray(_out)
    return (_out0, *[jnp.asarray(_g) for _g in _grads])
```

```python
import math
import jax
import jax.numpy as jnp
import jax.experimental.pallas as pl
import jax.experimental.pallas.tpu as pltpu

L = 2048
D = 576
N = 128
FH = 2304
B = 128
NB = L // B
TM = 256
EPS = 1e-5
F32 = jnp.float32
BF = jnp.bfloat16
HI = jax.lax.Precision.HIGHEST
GC = math.sqrt(2.0 / math.pi)


def _nn(a, b, prec=None):
    return jax.lax.dot_general(a, b, (((1,), (0,)), ((), ())), precision=prec,
                               preferred_element_type=F32)


def _nt(a, b, prec=None):
    return jax.lax.dot_general(a, b, (((1,), (1,)), ((), ())), precision=prec,
                               preferred_element_type=F32)


def _tn(a, b, prec=None):
    return jax.lax.dot_general(a, b, (((0,), (0,)), ((), ())), precision=prec,
                               preferred_element_type=F32)


def _ln(v):
    m = jnp.mean(v, axis=-1, keepdims=True)
    c = v - m
    var = jnp.mean(c * c, axis=-1, keepdims=True)
    r = jax.lax.rsqrt(var + EPS)
    return c * r, r


def _ln_bwd(dy, yhat, r):
    return r * (dy - jnp.mean(dy, axis=-1, keepdims=True)
                - yhat * jnp.mean(dy * yhat, axis=-1, keepdims=True))


def _gelu_parts(v):
    t = jnp.tanh(GC * (v + 0.044715 * v * v * v))
    g = 0.5 * v * (1.0 + t)
    dg = 0.5 * (1.0 + t) + 0.5 * v * (1.0 - t * t) * GC * (1.0 + 3 * 0.044715 * v * v)
    return g, dg


def _cexp(lr, li, pos):
    mag = jnp.exp(lr * pos)
    ang = li * pos
    return mag * jnp.cos(ang), mag * jnp.sin(ang)


def _iota(shape, dim):
    return jax.lax.broadcasted_iota(jnp.int32, shape, dim)


def _rows(i, n):
    return pl.ds(pl.multiple_of(i * n, n), n)


def _kernel(x_ref, are_ref, aim_ref, bre_ref, bim_ref, cre_ref, cim_ref, ldt_ref, dsk_ref,
            win_ref, wsp_ref, bsp_ref, wout_ref, g_ref,
            h2_ref, dx_ref, dare_ref, daim_ref, dbre_ref, dbim_ref, dcre_ref, dcim_ref,
            dldt_ref, ddsk_ref, dwin_ref, dwsp_ref, dbsp_ref, dwout_ref,
            f_ref, ft_ref, fq_ref, rh_ref, uf_ref, kf_ref, h_ref, hn_ref):

    def dft_t():
        k = ((2 * _iota((B, B), 1) + 1) * _iota((B, B), 0)) % (4 * B)
        ang = k.astype(F32) * (math.pi / (2 * B))
        return jnp.cos(ang), jnp.sin(ang)

    def dft_f():
        k = ((2 * _iota((B, B), 0) + 1) * _iota((B, B), 1)) % (4 * B)
        ang = k.astype(F32) * (math.pi / (2 * B))
        return jnp.cos(ang), jnp.sin(ang)

    cf, sf = dft_f()
    fmat = jnp.concatenate([cf, -sf], axis=0)
    f_ref[...] = fmat.astype(BF)
    ct, st = dft_t()
    ft_ref[...] = jnp.concatenate([ct, -st], axis=1).astype(BF)
    for o in range(4):
        base = (0, 256, 512, 1024)[o]
        lpos = (_iota((B, 2 * B), 0) + base).astype(F32)
        q = lpos.astype(BF).astype(F32) - float(base)
        sel = (q == _iota((B, 2 * B), 1).astype(F32)).astype(F32)
        fq_ref[o] = _nn(fmat, sel, HI).astype(BF)

    def octave(hi):
        return 0 if hi < 2 else (1 if hi < 4 else (2 if hi < 8 else 3))

    def p1(a, c):
        xv = x_ref[_rows(a, B), :].astype(F32)
        xn, r = _ln(xv)
        uf_ref[a] = _nn(f_ref[...], xn.astype(BF)).astype(BF)
        return c
    jax.lax.fori_loop(0, NB, p1, 0)

    def ssm_tabs(d):
        dt = jnp.exp(ldt_ref[pl.ds(d, 1), :].astype(F32)).astype(BF).astype(F32)
        lr = dt * are_ref[pl.ds(d, 1), :].astype(F32)
        li = dt * aim_ref[pl.ds(d, 1), :].astype(F32)
        e1r, e1i = _cexp(lr, li, _iota((8, 1), 0).astype(F32))
        e8r, e8i = _cexp(lr, li, (8 * _iota((16, 1), 0)).astype(F32))
        ehr, ehi = _cexp(lr, li, (B * _iota((24, 1), 0)).astype(F32))
        pr = (e8r[:, None, :] * e1r[None] - e8i[:, None, :] * e1i[None]).reshape(B, N)
        pi = (e8r[:, None, :] * e1i[None] + e8i[:, None, :] * e1r[None]).reshape(B, N)
        br = dt * bre_ref[pl.ds(d, 1), :].astype(F32)
        bi = dt * bim_ref[pl.ds(d, 1), :].astype(F32)
        cr = cre_ref[pl.ds(d, 1), :].astype(F32)
        ci = cim_ref[pl.ds(d, 1), :].astype(F32)
        return dt, pr, pi, ehr, ehi, br, bi, cr, ci

    def s4_fwd(kex_ref, yf_ref):
        def kgen(d, c):
            dt, pr, pi, ehr, ehi, br, bi, cr, ci = ssm_tabs(d)
            cbr = cr * br - ci * bi
            cbi = cr * bi + ci * br
            ar = cbr * ehr - cbi * ehi
            ai = cbr * ehi + cbi * ehr
            kex_ref[d] = _nt(jnp.concatenate([ar, -ai], axis=1),
                             jnp.concatenate([pr, pi], axis=1), HI)
            return c
        jax.lax.fori_loop(0, D, kgen, 0)
        for hi in range(NB):
            kw = jnp.concatenate([kex_ref[:, hi, :], kex_ref[:, hi + 1, :]], axis=1).astype(BF)
            kf_ref[hi] = _nt(fq_ref[octave(hi)], kw).astype(BF)

        sgn = jnp.where(_iota((B, 1), 0) % 2 == 0, 1.0, -1.0).astype(F32)

        def conv(a, carry):
            pyr, pyi = carry

            def mac(dl, acc):
                yr, yi = acc
                kr = kf_ref[dl, :B, :].astype(F32)
                ki = kf_ref[dl, B:, :].astype(F32)
                ur = uf_ref[a - dl, :B, :].astype(F32)
                ui = uf_ref[a - dl, B:, :].astype(F32)
                return yr + kr * ur - ki * ui, yi + kr * ui + ki * ur
            z = jnp.zeros((B, D), F32)
            yr, yi = jax.lax.fori_loop(0, a + 1, mac, (z, z))
            zc = jnp.concatenate([yr - sgn * pyi, yi + sgn * pyr], axis=0).astype(BF)
            y = _nn(ft_ref[...], zc) * (1.0 / B)
            xv = x_ref[_rows(a, B), :].astype(F32)
            xn, _ = _ln(xv)
            hv = xv + y + xn * dsk_ref[...].astype(F32)
            h_ref[_rows(a, B), :] = hv
            hn, r = _ln(hv)
            hn_ref[_rows(a, B), :] = hn.astype(BF)
            rh_ref[_rows(a, B), :] = r
            return yr, yi
        z0 = jnp.zeros((B, D), F32)
        jax.lax.fori_loop(0, NB, conv, (z0, z0))

    pl.run_scoped(s4_fwd, pltpu.VMEM((D, 24, N), F32), pltpu.VMEM((8, 128), F32))

    def gmlp(zp_ref, z2_ref, dg_ref, r2_ref, hnt_ref, dwot_ref):
        NT_ = L // TM

        def p4(t, c):
            rows = _rows(t, TM)
            hn = hn_ref[rows, :]
            hnt_ref[:, rows] = hn.astype(F32).T.astype(BF)
            zp = _nn(hn, win_ref[...]).astype(BF)
            zp_ref[rows, :] = zp
            z2g, _ = _gelu_parts(zp[:, FH:].astype(F32))
            z2, r = _ln(z2g)
            z2_ref[rows, :] = z2.astype(BF)
            r2_ref[rows, :] = r
            return c
        jax.lax.fori_loop(0, NT_, p4, 0)

        dwot_ref[...] = jnp.zeros_like(dwot_ref)

        def p5(t, c):
            rows = _rows(t, TM)
            g = _nn(wsp_ref[rows, :], z2_ref[...]) + bsp_ref[rows, :].astype(F32)
            z1, dz1g = _gelu_parts(zp_ref[rows, :FH].astype(F32))
            p = (z1 * g).astype(BF)
            gv = g_ref[rows, :]
            h2_ref[rows, :] = (h_ref[rows, :] + _nn(p, wout_ref[...])).astype(BF)
            dwot_ref[...] += _tn(p, gv)
            dp = _nt(gv, wout_ref[...])
            dg = dp * z1
            dbsp_ref[rows, :] = jnp.sum(dg, axis=-1, keepdims=True).astype(BF)
            dgb = dg.astype(BF)
            dg_ref[rows, :] = dgb
            zp_ref[rows, :FH] = (dp * g * dz1g).astype(BF)
            dwsp_ref[rows, :] = _nt(dgb, z2_ref[...]).astype(BF)
            return c
        jax.lax.fori_loop(0, NT_, p5, 0)
        dwout_ref[...] = dwot_ref[...].astype(BF)

        def p6(s, c):
            rows = _rows(s, TM)
            dz2 = _tn(wsp_ref[:, rows], dg_ref[...])
            dpre = _ln_bwd(dz2, z2_ref[rows, :].astype(F32), r2_ref[rows, :])
            _, dgel = _gelu_parts(zp_ref[rows, FH:].astype(F32))
            zp_ref[rows, FH:] = (dpre * dgel).astype(BF)
            dhn = _nt(zp_ref[rows, :], win_ref[...])
            dh = g_ref[rows, :].astype(F32) + _ln_bwd(dhn, hn_ref[rows, :].astype(F32),
                                                      rh_ref[rows, :])
            h_ref[rows, :] = dh
            return c
        jax.lax.fori_loop(0, NT_, p6, 0)

        CW = 512

        def p7(j, c):
            cols = pl.ds(pl.multiple_of(j * CW, CW), CW)
            dwin_ref[:, cols] = _nn(hnt_ref[...], zp_ref[:, cols]).astype(BF)
            return c
        jax.lax.fori_loop(0, 2 * FH // CW, p7, 0)

    pl.run_scoped(gmlp, pltpu.VMEM((L, 2 * FH), BF), pltpu.VMEM((L, FH), BF),
                  pltpu.VMEM((L, FH), BF), pltpu.VMEM((L, 1), F32),
                  pltpu.VMEM((D, L), BF), pltpu.VMEM((FH, D), F32))

    def s4_bwd(dkex_ref, dyf_ref, sg_ref, sl_ref):
        sgn = jnp.where(_iota((B, 1), 0) % 2 == 0, 1.0, -1.0).astype(F32)

        def pz(i, carry):
            nzr, nzi, acc = carry
            a = NB - 1 - i
            dy = h_ref[_rows(a, B), :]
            dz = _nn(f_ref[...], dy.astype(BF)) * (1.0 / B)
            zr, zi = dz[:B], dz[B:]
            dyf_ref[a, :B, :] = zr + sgn * nzi
            dyf_ref[a, B:, :] = zi - sgn * nzr
            xn, _ = _ln(x_ref[_rows(a, B), :].astype(F32))
            return zr, zi, acc + jnp.sum(dy * xn, axis=0, keepdims=True)
        z0 = jnp.zeros((B, D), F32)
        _, _, dsk = jax.lax.fori_loop(0, NB, pz, (z0, z0, jnp.zeros((1, D), F32)))
        ddsk_ref[...] = dsk.astype(BF)

        def pdu(b, c):
            def mac(dl, acc):
                ar_, ai_ = acc
                kr = kf_ref[dl, :B, :].astype(F32)
                ki = kf_ref[dl, B:, :].astype(F32)
                yr = dyf_ref[b + dl, :B, :]
                yi = dyf_ref[b + dl, B:, :]
                return ar_ + kr * yr + ki * yi, ai_ + kr * yi - ki * yr
            ur, ui = jax.lax.fori_loop(0, NB - b, mac, (z0, z0))
            du = _nn(ft_ref[...], jnp.concatenate([ur, ui], axis=0).astype(BF))
            rows = _rows(b, B)
            dh = h_ref[rows, :]
            dxn = du + dh * dsk_ref[...].astype(F32)
            xn, rx = _ln(x_ref[rows, :].astype(F32))
            dx_ref[rows, :] = (dh + _ln_bwd(dxn, xn, rx)).astype(BF)
            return c
        jax.lax.fori_loop(0, NB, pdu, 0)

        dkex_ref[...] = jnp.zeros_like(dkex_ref)
        for dl in range(NB):
            def mac(b, acc, dl=dl):
                ar_, ai_ = acc
                ur = uf_ref[b, :B, :].astype(F32)
                ui = uf_ref[b, B:, :].astype(F32)
                yr = dyf_ref[b + dl, :B, :]
                yi = dyf_ref[b + dl, B:, :]
                return ar_ + ur * yr + ui * yi, ai_ + ur * yi - ui * yr
            kr, ki = jax.lax.fori_loop(0, NB - dl, mac, (z0, z0))
            dkf = jnp.concatenate([kr, ki], axis=0).astype(BF)
            dkw = _tn(dkf, fq_ref[octave(dl)])
            dkex_ref[:, dl, :] += dkw[:, :B]
            dkex_ref[:, dl + 1, :] += dkw[:, B:]

        def pgrad(d, c):
            dt, pr, pi, ehr, ehi, br, bi, cr, ci = ssm_tabs(d)
            lo = _iota((B, 1), 0).astype(F32)
            rhs = jnp.concatenate([pr, pi, lo * pr, lo * pi], axis=1)
            s = _nn(dkex_ref[d], rhs, HI)
            sr, si, tr, ti = s[:, :N], s[:, N:2 * N], s[:, 2 * N:3 * N], s[:, 3 * N:]
            hb = (B * _iota((24, 1), 0)).astype(F32)
            tr = tr + hb * sr
            ti = ti + hb * si
            wr = jnp.sum(ehr * sr - ehi * si, axis=0, keepdims=True)
            wi = jnp.sum(ehr * si + ehi * sr, axis=0, keepdims=True)
            w2r = jnp.sum(ehr * tr - ehi * ti, axis=0, keepdims=True)
            w2i = jnp.sum(ehr * ti + ehi * tr, axis=0, keepdims=True)
            cbr = cr * br - ci * bi
            cbi = cr * bi + ci * br
            dcbr, dcbi = wr, -wi
            row = pl.ds(d, 1)
            sg_ref[4, row, :] = (dcbr * br + dcbi * bi)
            sg_ref[5, row, :] = (dcbi * br - dcbr * bi)
            ddbr = dcbr * cr + dcbi * ci
            ddbi = dcbi * cr - dcbr * ci
            sg_ref[2, row, :] = (dt * ddbr)
            sg_ref[3, row, :] = (dt * ddbi)
            dlr = cbr * w2r - cbi * w2i
            dli = -(cbr * w2i + cbi * w2r)
            sg_ref[0, row, :] = (dt * dlr)
            sg_ref[1, row, :] = (dt * dli)
            ddt = jnp.sum(ddbr * br + ddbi * bi
                          + dt * (dlr * are_ref[row, :].astype(F32)
                                  + dli * aim_ref[row, :].astype(F32)),
                          axis=-1, keepdims=True)
            sl_ref[row, :] = ddt
            return c
        jax.lax.fori_loop(0, D, pgrad, 0)
        for i, r in enumerate((dare_ref, daim_ref, dbre_ref, dbim_ref, dcre_ref, dcim_ref)):
            r[...] = sg_ref[i].astype(BF)
        dldt_ref[...] = sl_ref[...].astype(BF)

    pl.run_scoped(s4_bwd, pltpu.VMEM((D, 24, N), F32), pltpu.VMEM((NB, 2 * B, D), F32),
                  pltpu.VMEM((6, D, N), F32), pltpu.VMEM((D, 1), F32))


@jax.jit
def pallas_sequential_preLN__ssm_conv_s4__mixer_gmlp__prompt_kernel(
    A_u, A_A_re, A_A_im, A_B_re, A_B_im, A_C_re, A_C_im, A_log_dt, A_Dskip,
    B_x, B_w_in, B_w_sp, B_b_sp, B_w_out, grad_out,
):
    sd = lambda *s: jax.ShapeDtypeStruct(s, BF)
    out_shape = (sd(L, D), sd(L, D)) + (sd(D, N),) * 6 + (
        sd(D, 1), sd(1, D), sd(D, 2 * FH), sd(L, L), sd(L, 1), sd(FH, D))
    scratch = [
        pltpu.VMEM((2 * B, B), BF), pltpu.VMEM((B, 2 * B), BF), pltpu.VMEM((4, 2 * B, 2 * B), BF),
        pltpu.VMEM((L, 1), F32),
        pltpu.VMEM((NB, 2 * B, D), BF), pltpu.VMEM((NB, 2 * B, D), BF),
        pltpu.VMEM((L, D), F32), pltpu.VMEM((L, D), BF),
    ]
    vm = pl.BlockSpec(memory_space=pltpu.VMEM)
    outs = pl.pallas_call(
        _kernel,
        out_shape=out_shape,
        in_specs=[vm] * 14,
        out_specs=tuple([vm] * 14),
        scratch_shapes=scratch,
        compiler_params=pltpu.CompilerParams(vmem_limit_bytes=127 * 1024 * 1024),
    )(A_u.reshape(L, D), A_A_re.astype(F32), A_A_im.astype(F32), A_B_re.astype(F32),
      A_B_im.astype(F32), A_C_re.astype(F32), A_C_im.astype(F32),
      A_log_dt.reshape(D, 1).astype(F32), A_Dskip.reshape(1, D), B_w_in, B_w_sp,
      B_b_sp.reshape(L, 1), B_w_out, grad_out.reshape(L, D))
    (h2, dx, dare, daim, dbre, dbim, dcre, dcim, dldt, ddsk, dwin, dwsp, dbsp, dwout) = outs
    return (h2.reshape(1, L, D), dx.reshape(1, L, D), dare, daim, dbre, dbim, dcre, dcim,
            dldt.reshape(D), ddsk.reshape(D), dwin, dwsp, dbsp.reshape(L), dwout)
```

```python
import math
import jax
import jax.numpy as jnp
import jax.experimental.pallas as pl
import jax.experimental.pallas.tpu as pltpu

L = 2048
D = 576
N = 128
FH = 2304
B = 128
NB = L // B
TM = 256
EPS = 1e-5
F32 = jnp.float32
BF = jnp.bfloat16
HI = jax.lax.Precision.HIGHEST
GC = math.sqrt(2.0 / math.pi)


def _nn(a, b, prec=None):
    return jax.lax.dot_general(a, b, (((1,), (0,)), ((), ())), precision=prec,
                               preferred_element_type=F32)


def _nt(a, b, prec=None):
    return jax.lax.dot_general(a, b, (((1,), (1,)), ((), ())), precision=prec,
                               preferred_element_type=F32)


def _tn(a, b, prec=None):
    return jax.lax.dot_general(a, b, (((0,), (0,)), ((), ())), precision=prec,
                               preferred_element_type=F32)


def _ln(v):
    m = jnp.mean(v, axis=-1, keepdims=True)
    c = v - m
    var = jnp.mean(c * c, axis=-1, keepdims=True)
    r = jax.lax.rsqrt(var + EPS)
    return c * r, r


def _ln_bwd(dy, yhat, r):
    return r * (dy - jnp.mean(dy, axis=-1, keepdims=True)
                - yhat * jnp.mean(dy * yhat, axis=-1, keepdims=True))


def _gelu_parts(v):
    t = jnp.tanh(GC * (v + 0.044715 * v * v * v))
    g = 0.5 * v * (1.0 + t)
    dg = 0.5 * (1.0 + t) + 0.5 * v * (1.0 - t * t) * GC * (1.0 + 3 * 0.044715 * v * v)
    return g, dg


def _cexp(lr, li, pos):
    mag = jnp.exp(lr * pos)
    ang = li * pos
    return mag * jnp.cos(ang), mag * jnp.sin(ang)


def _iota(shape, dim):
    return jax.lax.broadcasted_iota(jnp.int32, shape, dim)


def _rows(i, n):
    return pl.ds(pl.multiple_of(i * n, n), n)


CH = 32


def _cmac(n, aref, aidx, bref, bidx, conj_a):
    outs_r, outs_i = [], []
    for c in range(B // CH):
        lo, hi = c * CH, B + c * CH

        def body(i, acc):
            r, m = acc
            ar = aref[aidx(i), lo:lo + CH, :].astype(F32)
            ai = aref[aidx(i), hi:hi + CH, :].astype(F32)
            br = bref[bidx(i), lo:lo + CH, :].astype(F32)
            bi = bref[bidx(i), hi:hi + CH, :].astype(F32)
            if conj_a:
                return r + ar * br + ai * bi, m + ar * bi - ai * br
            return r + ar * br - ai * bi, m + ar * bi + ai * br
        z = jnp.zeros((CH, D), F32)
        r, m = jax.lax.fori_loop(0, n, body, (z, z))
        outs_r.append(r)
        outs_i.append(m)
    return jnp.concatenate(outs_r, axis=0), jnp.concatenate(outs_i, axis=0)


def _kernel(x_ref, are_ref, aim_ref, bre_ref, bim_ref, cre_ref, cim_ref, ldt_ref, dsk_ref,
            win_hbm, wsp_hbm, bsp_ref, wout_hbm, g_ref,
            h2_ref, dx_ref, dare_ref, daim_ref, dbre_ref, dbim_ref, dcre_ref, dcim_ref,
            dldt_ref, ddsk_ref, dwin_hbm, dwsp_hbm, dbsp_ref, dwout_hbm,
            f_ref, ft_ref, fq_ref, rh_ref, uf_ref, kf_ref, h_ref, hn_ref,
            win_ref, wsp_ref, wout_ref, dwin_ref, dwsp_ref, dwout_ref, sems):

    cp_in = [pltpu.make_async_copy(a, b, sems.at[i]) for i, (a, b) in enumerate(
        ((win_hbm, win_ref), (wsp_hbm, wsp_ref), (wout_hbm, wout_ref)))]
    cp_out = [pltpu.make_async_copy(a, b, sems.at[3 + i]) for i, (a, b) in enumerate(
        ((dwsp_ref, dwsp_hbm), (dwout_ref, dwout_hbm), (dwin_ref, dwin_hbm)))]
    for cp in cp_in:
        cp.start()

    def dft_t():
        k = ((2 * _iota((B, B), 1) + 1) * _iota((B, B), 0)) % (4 * B)
        ang = k.astype(F32) * (math.pi / (2 * B))
        return jnp.cos(ang), jnp.sin(ang)

    def dft_f():
        k = ((2 * _iota((B, B), 0) + 1) * _iota((B, B), 1)) % (4 * B)
        ang = k.astype(F32) * (math.pi / (2 * B))
        return jnp.cos(ang), jnp.sin(ang)

    cf, sf = dft_f()
    fmat = jnp.concatenate([cf, -sf], axis=0)
    f_ref[...] = fmat.astype(BF)
    ct, st = dft_t()
    ft_ref[...] = jnp.concatenate([ct, -st], axis=1).astype(BF)
    for o in range(4):
        base = (0, 256, 512, 1024)[o]
        lpos = (_iota((B, 2 * B), 0) + base).astype(F32)
        q = lpos.astype(BF).astype(F32) - float(base)
        sel = (q == _iota((B, 2 * B), 1).astype(F32)).astype(F32)
        fq_ref[o] = _nn(fmat, sel, HI).astype(BF)

    def octave(hi):
        return 0 if hi < 2 else (1 if hi < 4 else (2 if hi < 8 else 3))

    def p1(a, c):
        xv = x_ref[_rows(a, B), :].astype(F32)
        xn, r = _ln(xv)
        uf_ref[a] = _nn(f_ref[...], xn.astype(BF)).astype(BF)
        return c
    with jax.named_scope('p1'):
        jax.lax.fori_loop(0, NB, p1, 0)

    def ssm_tabs(d):
        dt = jnp.exp(ldt_ref[pl.ds(d, 1), :].astype(F32)).astype(BF).astype(F32)
        lr = dt * are_ref[pl.ds(d, 1), :].astype(F32)
        li = dt * aim_ref[pl.ds(d, 1), :].astype(F32)
        pwr, pwi = _cexp(lr, li, jnp.left_shift(1, _iota((16, 1), 0)).astype(F32))

        def table(nrows, k0, nbits):
            rid = _iota((nrows, 1), 0)
            tr = ti = None
            for j in range(nbits):
                bit = (jnp.right_shift(rid, j) & 1) == 1
                fr = jnp.where(bit, pwr[k0 + j:k0 + j + 1, :], 1.0)
                fi = jnp.where(bit, pwi[k0 + j:k0 + j + 1, :], 0.0)
                if tr is None:
                    tr, ti = fr, fi
                else:
                    tr, ti = tr * fr - ti * fi, tr * fi + ti * fr
            return tr, ti
        e1r, e1i = table(8, 0, 3)
        e8r, e8i = table(16, 3, 4)
        ehr, ehi = table(24, 7, 5)
        pr = (e8r[:, None, :] * e1r[None] - e8i[:, None, :] * e1i[None]).reshape(B, N)
        pi = (e8r[:, None, :] * e1i[None] + e8i[:, None, :] * e1r[None]).reshape(B, N)
        br = dt * bre_ref[pl.ds(d, 1), :].astype(F32)
        bi = dt * bim_ref[pl.ds(d, 1), :].astype(F32)
        cr = cre_ref[pl.ds(d, 1), :].astype(F32)
        ci = cim_ref[pl.ds(d, 1), :].astype(F32)
        return dt, pr, pi, ehr, ehi, br, bi, cr, ci

    def s4_fwd(kex_ref, yf_ref):
        def kgen(d, c):
            dt, pr, pi, ehr, ehi, br, bi, cr, ci = ssm_tabs(d)
            cbr = cr * br - ci * bi
            cbi = cr * bi + ci * br
            ar = cbr * ehr - cbi * ehi
            ai = cbr * ehi + cbi * ehr
            kex_ref[d] = _nt(jnp.concatenate([ar, -ai], axis=1),
                             jnp.concatenate([pr, pi], axis=1), jax.lax.Precision.HIGH)
            return c
        with jax.named_scope('kgen'):
            jax.lax.fori_loop(0, D, kgen, 0, unroll=8)
        for hi in range(NB):
            kw = jnp.concatenate([kex_ref[:, hi, :], kex_ref[:, hi + 1, :]], axis=1).astype(BF)
            kf_ref[hi] = _nt(fq_ref[octave(hi)], kw).astype(BF)

        sgn = jnp.where(_iota((B, 1), 0) % 2 == 0, 1.0, -1.0).astype(F32)

        def conv(a, carry):
            pyr, pyi = carry

            yr, yi = _cmac(a + 1, kf_ref, lambda i: i, uf_ref, lambda i: a - i, False)
            zc = jnp.concatenate([yr - sgn * pyi, yi + sgn * pyr], axis=0).astype(BF)
            y = _nn(ft_ref[...], zc) * (1.0 / B)
            xv = x_ref[_rows(a, B), :].astype(F32)
            xn, _ = _ln(xv)
            hv = xv + y + xn * dsk_ref[...].astype(F32)
            h_ref[_rows(a, B), :] = hv
            hn, r = _ln(hv)
            hn_ref[_rows(a, B), :] = hn.astype(BF)
            rh_ref[_rows(a, B), :] = r
            return yr, yi
        z0 = jnp.zeros((B, D), F32)
        with jax.named_scope('conv'):
            jax.lax.fori_loop(0, NB, conv, (z0, z0))

    pl.run_scoped(s4_fwd, pltpu.VMEM((D, 24, N), F32), pltpu.VMEM((8, 128), F32))

    def gmlp(zp_ref, z2_ref, dg_ref, r2_ref, hnt_ref, dwot_ref):
        NT_ = L // TM
        for cp in cp_in:
            cp.wait()

        def p4(t, c):
            rows = _rows(t, TM)
            hn = hn_ref[rows, :]
            hnt_ref[:, rows] = hn.astype(F32).T.astype(BF)
            zp = _nn(hn, win_ref[...]).astype(BF)
            zp_ref[rows, :] = zp
            z2g, _ = _gelu_parts(zp[:, FH:].astype(F32))
            z2, r = _ln(z2g)
            z2_ref[rows, :] = z2.astype(BF)
            r2_ref[rows, :] = r
            return c
        with jax.named_scope('p4'):
            jax.lax.fori_loop(0, NT_, p4, 0)

        dwot_ref[...] = jnp.zeros_like(dwot_ref)

        def p5(t, c):
            rows = _rows(t, TM)
            g = _nn(wsp_ref[rows, :], z2_ref[...]) + bsp_ref[rows, :].astype(F32)
            z1, dz1g = _gelu_parts(zp_ref[rows, :FH].astype(F32))
            p = (z1 * g).astype(BF)
            gv = g_ref[rows, :]
            h2_ref[rows, :] = (h_ref[rows, :] + _nn(p, wout_ref[...])).astype(BF)
            dwot_ref[...] += _tn(p, gv)
            dp = _nt(gv, wout_ref[...])
            dg = dp * z1
            dbsp_ref[rows, :] = jnp.sum(dg, axis=-1, keepdims=True).astype(BF)
            dgb = dg.astype(BF)
            dg_ref[rows, :] = dgb
            zp_ref[rows, :FH] = (dp * g * dz1g).astype(BF)
            dwsp_ref[rows, :] = _nt(dgb, z2_ref[...]).astype(BF)
            return c
        with jax.named_scope('p5'):
            jax.lax.fori_loop(0, NT_, p5, 0)
        dwout_ref[...] = dwot_ref[...].astype(BF)
        cp_out[0].start()
        cp_out[1].start()

        def p6(s, c):
            rows = _rows(s, TM)
            dz2 = _tn(wsp_ref[:, rows], dg_ref[...])
            dpre = _ln_bwd(dz2, z2_ref[rows, :].astype(F32), r2_ref[rows, :])
            _, dgel = _gelu_parts(zp_ref[rows, FH:].astype(F32))
            zp_ref[rows, FH:] = (dpre * dgel).astype(BF)
            dhn = _nt(zp_ref[rows, :], win_ref[...])
            dh = g_ref[rows, :].astype(F32) + _ln_bwd(dhn, hn_ref[rows, :].astype(F32),
                                                      rh_ref[rows, :])
            h_ref[rows, :] = dh
            return c
        with jax.named_scope('p6'):
            jax.lax.fori_loop(0, NT_, p6, 0)

        CW = 512

        def p7(j, c):
            cols = pl.ds(pl.multiple_of(j * CW, CW), CW)
            dwin_ref[:, cols] = _nn(hnt_ref[...], zp_ref[:, cols]).astype(BF)
            return c
        with jax.named_scope('p7'):
            jax.lax.fori_loop(0, 2 * FH // CW, p7, 0)
        cp_out[2].start()

    pl.run_scoped(gmlp, pltpu.VMEM((L, 2 * FH), BF), pltpu.VMEM((L, FH), BF),
                  pltpu.VMEM((L, FH), BF), pltpu.VMEM((L, 1), F32),
                  pltpu.VMEM((D, L), BF), pltpu.VMEM((FH, D), F32))

    def s4_bwd(dkex_ref, dyf_ref, sg_ref, sl_ref):
        sgn = jnp.where(_iota((B, 1), 0) % 2 == 0, 1.0, -1.0).astype(F32)

        def pz(i, carry):
            nzr, nzi, acc = carry
            a = NB - 1 - i
            dy = h_ref[_rows(a, B), :]
            dz = _nn(f_ref[...], dy.astype(BF)) * (1.0 / B)
            zr, zi = dz[:B], dz[B:]
            dyf_ref[a, :B, :] = zr + sgn * nzi
            dyf_ref[a, B:, :] = zi - sgn * nzr
            xn, _ = _ln(x_ref[_rows(a, B), :].astype(F32))
            return zr, zi, acc + jnp.sum(dy * xn, axis=0, keepdims=True)
        z0 = jnp.zeros((B, D), F32)
        with jax.named_scope('pz'):
            _, _, dsk = jax.lax.fori_loop(0, NB, pz, (z0, z0, jnp.zeros((1, D), F32)))
        ddsk_ref[...] = dsk.astype(BF)

        def pdu(b, c):
            ur, ui = _cmac(NB - b, kf_ref, lambda i: i, dyf_ref, lambda i: b + i, True)
            du = _nn(ft_ref[...], jnp.concatenate([ur, ui], axis=0).astype(BF))
            rows = _rows(b, B)
            dh = h_ref[rows, :]
            dxn = du + dh * dsk_ref[...].astype(F32)
            xn, rx = _ln(x_ref[rows, :].astype(F32))
            dx_ref[rows, :] = (dh + _ln_bwd(dxn, xn, rx)).astype(BF)
            return c
        with jax.named_scope('pdu'):
            jax.lax.fori_loop(0, NB, pdu, 0)

        dkex_ref[...] = jnp.zeros_like(dkex_ref)
        for dl in range(NB):
          with jax.named_scope('pdk'):
              kr, ki = _cmac(NB - dl, uf_ref, lambda i: i, dyf_ref, lambda i, dl=dl: i + dl, True)
              dkf = jnp.concatenate([kr, ki], axis=0).astype(BF)
              dkw = _tn(dkf, fq_ref[octave(dl)])
              dkex_ref[:, dl, :] += dkw[:, :B]
              dkex_ref[:, dl + 1, :] += dkw[:, B:]

        def pgrad(d, c):
            dt, pr, pi, ehr, ehi, br, bi, cr, ci = ssm_tabs(d)
            lo = _iota((B, 1), 0).astype(F32)
            rhs = jnp.concatenate([pr, pi, lo * pr, lo * pi], axis=1)
            s = _nn(dkex_ref[d], rhs, jax.lax.Precision.HIGH)
            sr, si, tr, ti = s[:, :N], s[:, N:2 * N], s[:, 2 * N:3 * N], s[:, 3 * N:]
            hb = (B * _iota((24, 1), 0)).astype(F32)
            tr = tr + hb * sr
            ti = ti + hb * si
            wr = jnp.sum(ehr * sr - ehi * si, axis=0, keepdims=True)
            wi = jnp.sum(ehr * si + ehi * sr, axis=0, keepdims=True)
            w2r = jnp.sum(ehr * tr - ehi * ti, axis=0, keepdims=True)
            w2i = jnp.sum(ehr * ti + ehi * tr, axis=0, keepdims=True)
            cbr = cr * br - ci * bi
            cbi = cr * bi + ci * br
            dcbr, dcbi = wr, -wi
            row = pl.ds(d, 1)
            sg_ref[4, row, :] = (dcbr * br + dcbi * bi)
            sg_ref[5, row, :] = (dcbi * br - dcbr * bi)
            ddbr = dcbr * cr + dcbi * ci
            ddbi = dcbi * cr - dcbr * ci
            sg_ref[2, row, :] = (dt * ddbr)
            sg_ref[3, row, :] = (dt * ddbi)
            dlr = cbr * w2r - cbi * w2i
            dli = -(cbr * w2i + cbi * w2r)
            sg_ref[0, row, :] = (dt * dlr)
            sg_ref[1, row, :] = (dt * dli)
            ddt = jnp.sum(ddbr * br + ddbi * bi
                          + dt * (dlr * are_ref[row, :].astype(F32)
                                  + dli * aim_ref[row, :].astype(F32)),
                          axis=-1, keepdims=True)
            sl_ref[row, :] = ddt
            return c
        with jax.named_scope('pgrad'):
            jax.lax.fori_loop(0, D, pgrad, 0, unroll=8)
        for i, r in enumerate((dare_ref, daim_ref, dbre_ref, dbim_ref, dcre_ref, dcim_ref)):
            r[...] = sg_ref[i].astype(BF)
        dldt_ref[...] = sl_ref[...].astype(BF)

    pl.run_scoped(s4_bwd, pltpu.VMEM((D, 24, N), F32), pltpu.VMEM((NB, 2 * B, D), F32),
                  pltpu.VMEM((6, D, N), F32), pltpu.VMEM((D, 1), F32))
    for cp in cp_out:
        cp.wait()


@jax.jit
def pallas_sequential_preLN__ssm_conv_s4__mixer_gmlp__prompt_kernel(
    A_u, A_A_re, A_A_im, A_B_re, A_B_im, A_C_re, A_C_im, A_log_dt, A_Dskip,
    B_x, B_w_in, B_w_sp, B_b_sp, B_w_out, grad_out,
):
    sd = lambda *s: jax.ShapeDtypeStruct(s, BF)
    out_shape = (sd(L, D), sd(L, D)) + (sd(D, N),) * 6 + (
        sd(D, 1), sd(1, D), sd(D, 2 * FH), sd(L, L), sd(L, 1), sd(FH, D))
    scratch = [
        pltpu.VMEM((2 * B, B), BF), pltpu.VMEM((B, 2 * B), BF), pltpu.VMEM((4, 2 * B, 2 * B), BF),
        pltpu.VMEM((L, 1), F32),
        pltpu.VMEM((NB, 2 * B, D), BF), pltpu.VMEM((NB, 2 * B, D), BF),
        pltpu.VMEM((L, D), F32), pltpu.VMEM((L, D), BF),
        pltpu.VMEM((D, 2 * FH), BF), pltpu.VMEM((L, L), BF), pltpu.VMEM((FH, D), BF),
        pltpu.VMEM((D, 2 * FH), BF), pltpu.VMEM((L, L), BF), pltpu.VMEM((FH, D), BF),
        pltpu.SemaphoreType.DMA((6,)),
    ]
    vm = pl.BlockSpec(memory_space=pltpu.VMEM)
    hb = pl.BlockSpec(memory_space=pl.ANY)
    outs = pl.pallas_call(
        _kernel,
        out_shape=out_shape,
        in_specs=[vm] * 9 + [hb, hb, vm, hb, vm],
        out_specs=tuple([vm] * 10 + [hb, hb, vm, hb]),
        scratch_shapes=scratch,
        compiler_params=pltpu.CompilerParams(vmem_limit_bytes=127 * 1024 * 1024),
    )(A_u.reshape(L, D), A_A_re.astype(F32), A_A_im.astype(F32), A_B_re.astype(F32),
      A_B_im.astype(F32), A_C_re.astype(F32), A_C_im.astype(F32),
      A_log_dt.reshape(D, 1).astype(F32), A_Dskip.reshape(1, D), B_w_in, B_w_sp,
      B_b_sp.reshape(L, 1), B_w_out, grad_out.reshape(L, D))
    (h2, dx, dare, daim, dbre, dbim, dcre, dcim, dldt, ddsk, dwin, dwsp, dbsp, dwout) = outs
    return (h2.reshape(1, L, D), dx.reshape(1, L, D), dare, daim, dbre, dbim, dcre, dcim,
            dldt.reshape(D), ddsk.reshape(D), dwin, dwsp, dbsp.reshape(L), dwout)
```
